```python
import os as _os
_os.environ.setdefault("JAX_PLATFORMS", "cpu")
import jax
import jax.numpy as jnp

def _softmax(x, axis=-1):
    return jax.nn.softmax(x, axis=axis)
def _gelu(x):
    return jax.nn.gelu(x, approximate=True)
def _silu(x):
    return jax.nn.silu(x)
def _sigmoid(x):
    return jax.nn.sigmoid(x)
def _layernorm(x, axis=-1, eps=1e-5):
    m = jnp.mean(x, axis=axis, keepdims=True)
    v = jnp.var(x, axis=axis, keepdims=True)
    return (x - m) / jnp.sqrt(v + eps)
def _scatter_add(tgt, idx, src, axis=0):
    return tgt.at[idx].add(src)
def _segment_sum(src, seg, n):
    return jax.ops.segment_sum(src, seg, n)
class _Rng:
    def __init__(self, key):
        self._k = key
    def _next(self):
        self._k, sub = jax.random.split(self._k)
        return sub
    def normal(self, shape):
        return jax.random.normal(self._next(), shape, dtype=jnp.bfloat16)
    def randint(self, lo, hi, shape):
        return jax.random.randint(self._next(), shape, lo, hi, dtype=jnp.int32)
    def uniform(self, shape, lo=0.0, hi=1.0):
        return jax.random.uniform(self._next(), shape, jnp.bfloat16, lo, hi)
    def permutation(self, n):
        return jax.random.permutation(self._next(), n)


kernel_name = 'standalone__gqa_block_cached__sampling'

def setup_inputs():
    _rng = _Rng(jax.random.key(int.from_bytes(__import__("os").urandom(4), "little")))
    _w = (lambda a: (lambda t: t.astype(jnp.bfloat16) if jnp.issubdtype(t.dtype, jnp.floating) else t)(jnp.asarray(a)))
    B, Sq, D = 32, 16, 1024
    Hq, Hkv, Sk, Dh = 32, 4, 2048, 128
    assert Hq % Hkv == 0, (Hq, Hkv)
    return {
        "x": _w((lambda *s: _rng.normal(s) * 0.8)(B, Sq, D)),
        "k_cache": _w((lambda *s: _rng.normal(s) * 0.8)(B, Hkv, Sk, Dh)),
        "v_cache": _w((lambda *s: _rng.normal(s) * 0.05)(B, Hkv, Sk, Dh)),
        "wq": _w((lambda *s: _rng.normal(s) * 0.8)(D, Hq * Dh) * (D ** -0.5)),
        "wo": _w((lambda *s: _rng.normal(s) * 0.05)(Hq * Dh, D) * ((Hq * Dh) ** -0.5)),
    }

def reference(x, k_cache, v_cache, wq, wo):
    B, Sq, D = x.shape
    Hq, Dh = 32, 128
    Hkv = k_cache.shape[1]
    rep = Hq // Hkv
    q = (lambda x, *d: x.transpose(*d))((x @ wq).reshape(B, Sq, Hq, Dh), 0, 2, 1, 3)
    k = jnp.repeat(k_cache, rep, axis=1)
    v = jnp.repeat(v_cache, rep, axis=1)
    scores = jnp.einsum("bhqd,bhkd->bhqk", q, k) * (Dh ** -0.5)
    p = _softmax(scores, axis=-1)
    o = jnp.einsum("bhqk,bhkd->bhqd", p, v)
    return (lambda x, *d: x.transpose(*d))(o, 0, 2, 1, 3).reshape(B, Sq, Hq * Dh) @ wo
```

```python
import functools
import jax
import jax.numpy as jnp
import numpy as np
import jax.experimental.pallas as pl
import jax.experimental.pallas.tpu as pltpu

LOG2E = 1.4426950408889634


def make(NSLOT=16, wo_at=4, wo0_after=8, defer=True, split_wait=True, small=True):
    def fn(x, k_cache, v_cache, wq, wo):
        B, Sq, D = x.shape
        _, Hkv, Sk, Dh = k_cache.shape
        Hq = wq.shape[1] // Dh
        rep = Hq // Hkv
        G = rep * Dh
        M = B * Sq
        N = B * Hkv
        BB = 2
        ND = N // BB
        DPP = B // BB
        CB = 8
        DPC = CB // BB
        CR = CB * Sq
        NC = B // CB
        qscale = float(Dh ** -0.5 * LOG2E)
        assert NSLOT % BB == 0

        def kernel(x_hbm, k_hbm, v_hbm, wq_hbm, wo_hbm, o_hbm,
                   kb, vb, xb, wqb, wob, q_s, o_s, acc_s, ob, ksem, vsem, wqsem, wosem, xsem, osem):
            def kv_copies(i, slot):
                g = i // B
                b = i % B
                return (pltpu.make_async_copy(k_hbm.at[b, g], kb.at[slot], ksem.at[slot]),
                        pltpu.make_async_copy(v_hbm.at[b, g], vb.at[slot], vsem.at[slot]))

            def kv_start(i, slot):
                ck, cv = kv_copies(i, slot)
                ck.start()
                cv.start()

            def wq_copy(g):
                return pltpu.make_async_copy(wq_hbm.at[:, pl.ds(pl.multiple_of(g * G, G), G)], wqb.at[g], wqsem.at[g])

            def wo_copy(g):
                return pltpu.make_async_copy(wo_hbm.at[pl.ds(pl.multiple_of(g * G, G), G), :], wob.at[g % 2], wosem.at[g % 2])

            def out_copy(r0, n, s):
                return pltpu.make_async_copy(ob.at[pl.ds(r0, n), :], o_hbm.at[pl.ds(r0, n), :], osem.at[s])

            cx = pltpu.make_async_copy(x_hbm, xb, xsem.at[0])
            cx.start()

            def w_fill(g, _):
                wq_copy(g).start()
                return 0
            jax.lax.fori_loop(0, Hkv, w_fill, 0)

            def fill(i, _):
                kv_start(i, i)
                return 0
            jax.lax.fori_loop(0, wo0_after, fill, 0)
            wo_copy(0).start()
            jax.lax.fori_loop(wo0_after, NSLOT, fill, 0)

            acc_s[...] = jnp.zeros_like(acc_s)
            cx.wait()

            def qproj(g, _):
                wq_copy(g).wait()
                q = jnp.dot(xb[...], wqb[g], preferred_element_type=jnp.float32)
                q_s[g] = (q * qscale).astype(jnp.bfloat16)
                return 0
            jax.lax.fori_loop(0, Hkv, qproj, 0)

            def attn(g, b, slot, wait_v):
                row0 = pl.multiple_of(b * Sq, Sq)
                qq = jnp.concatenate([q_s[g, pl.ds(row0, Sq), h * Dh:(h + 1) * Dh] for h in range(rep)], axis=0)
                k = kb[slot]
                s = jax.lax.dot_general(qq, k, (((1,), (1,)), ((), ())), preferred_element_type=jnp.float32)
                m = jnp.max(s, axis=1, keepdims=True)
                wait_v()
                p = jnp.exp2(s - m)
                l = jnp.sum(p, axis=1, keepdims=True)
                o = jnp.dot(p.astype(jnp.bfloat16), vb[slot], preferred_element_type=jnp.float32)
                o = o * pl.reciprocal(l, approx=False)
                ob_ = o.astype(jnp.bfloat16)
                orow = pl.multiple_of((b % CB) * Sq, Sq)
                for h in range(rep):
                    o_s[pl.ds(orow, Sq), h * Dh:(h + 1) * Dh] = ob_[h * Sq:(h + 1) * Sq, :]

            def duo(d, _):
                g = d // DPP
                dd = d % DPP
                i0 = d * BB
                s0 = pl.multiple_of(i0 % NSLOT, BB)

                @pl.when((dd == wo_at) & (g + 1 < Hkv))
                def _():
                    wo_copy(g + 1).start()

                cps = [kv_copies(i0 + j, s0 + j) for j in range(BB)]
                if not split_wait:
                    for ck, cv in cps:
                        ck.wait(); cv.wait()

                if defer:
                    @pl.when(d == ND - 1)
                    def _():
                        out_copy(0, M - BB * Sq if small else M - CR, 0).start()

                for j in range(BB):
                    if split_wait:
                        cps[j][0].wait()
                        attn(g, dd * BB + j, s0 + j, cps[j][1].wait)
                    else:
                        attn(g, dd * BB + j, s0 + j, lambda: None)

                @pl.when(i0 + NSLOT < N)
                def _():
                    for j in range(BB):
                        kv_start(i0 + j + NSLOT, s0 + j)

                @pl.when(dd == DPC - 1)
                def _():
                    wo_copy(g).wait()

                last_chunk = (d >= ND - DPC) if small else False
                big = (dd % DPC == DPC - 1)
                if small:
                    big = big & jnp.logical_not(last_chunk)

                @pl.when(big)
                def _():
                    r0 = pl.multiple_of((dd // DPC) * CR, CR)
                    a = acc_s[pl.ds(r0, CR), :] + jnp.dot(o_s[...], wob[g % 2], preferred_element_type=jnp.float32)
                    acc_s[pl.ds(r0, CR), :] = a
                    ob[pl.ds(r0, CR), :] = a.astype(ob.dtype)
                    if not defer:
                        @pl.when(g == Hkv - 1)
                        def _():
                            pltpu.make_async_copy(ob.at[pl.ds(r0, CR), :], o_hbm.at[pl.ds(r0, CR), :], osem.at[dd // DPC]).start()

                if small:
                    @pl.when(last_chunk)
                    def _():
                        r0 = pl.multiple_of(dd * BB * Sq, BB * Sq)
                        rs = pl.multiple_of((dd % DPC) * BB * Sq, BB * Sq)
                        a = acc_s[pl.ds(r0, BB * Sq), :] + jnp.dot(o_s[pl.ds(rs, BB * Sq), :], wob[(Hkv - 1) % 2], preferred_element_type=jnp.float32)
                        ob[pl.ds(r0, BB * Sq), :] = a.astype(ob.dtype)
                return 0

            jax.lax.fori_loop(0, ND, duo, 0)
            if defer:
                n = BB * Sq if small else CR
                c2 = out_copy(M - n, n, 1)
                c2.start()
                out_copy(0, M - n, 0).wait()
                c2.wait()
            else:
                if small:
                    c2 = out_copy(M - CR, CR, NC - 1)
                    c2.start()
                for c in range(NC):
                    out_copy(c * CR, CR, c).wait()

        out = pl.pallas_call(
            kernel,
            in_specs=[pl.BlockSpec(memory_space=pl.ANY)] * 5,
            out_specs=pl.BlockSpec(memory_space=pl.ANY),
            out_shape=jax.ShapeDtypeStruct((M, D), x.dtype),
            scratch_shapes=[
                pltpu.VMEM((NSLOT, Sk, Dh), jnp.bfloat16),
                pltpu.VMEM((NSLOT, Sk, Dh), jnp.bfloat16),
                pltpu.VMEM((M, D), jnp.bfloat16),
                pltpu.VMEM((Hkv, D, G), jnp.bfloat16),
                pltpu.VMEM((2, G, D), jnp.bfloat16),
                pltpu.VMEM((Hkv, M, G), jnp.bfloat16),
                pltpu.VMEM((CR, G), jnp.bfloat16),
                pltpu.VMEM((M, D), jnp.float32),
                pltpu.VMEM((M, D), jnp.bfloat16),
                pltpu.SemaphoreType.DMA((NSLOT,)),
                pltpu.SemaphoreType.DMA((NSLOT,)),
                pltpu.SemaphoreType.DMA((Hkv,)),
                pltpu.SemaphoreType.DMA((2,)),
                pltpu.SemaphoreType.DMA((1,)),
                pltpu.SemaphoreType.DMA((NC,)),
            ],
            compiler_params=pltpu.CompilerParams(vmem_limit_bytes=110 * 1024 * 1024),
        )(x.reshape(M, D), k_cache, v_cache, wq, wo)
        return out.reshape(B, Sq, D)
    return fn

pallas_standalone__gqa_block_cached__sampling_kernel = jax.jit(make())
```

```python
import contextlib
import jax
import jax.numpy as jnp
import numpy as np
import jax.experimental.pallas as pl
import jax.experimental.pallas.tpu as pltpu

LOG2E = 1.4426950408889634


def make(NSLOT=16, L1=None, LK=3, LV=2, wo_at=4, wo0_after=8, NPK=4, NPV=4, PROW=128, SCH=4, PCH=4, nobc=False,
         scopes=False, order="IAB", scheme="422", nodma=False, bigpos=0, tie=False, QN=8, QM=2, NQ=0, CH_S=0, WOP=True, ON=8, OPP=1, WQP=True, QPP=1, blast=True, kpos='after', vpos='after'):
    def fn(x, k_cache, v_cache, wq, wo):
        B, Sq, D = x.shape
        _, Hkv, Sk, Dh = k_cache.shape
        Hq = wq.shape[1] // Dh
        rep = Hq // Hkv
        G = rep * Dh
        M = B * Sq
        R = rep * Sq
        N = B * Hkv
        CB = 8
        CR = CB * Sq
        qscale = float(Dh ** -0.5 * LOG2E)
        kbig = Sk - NPK * PROW
        vbig = Sk - NPV * PROW
        LOOK = (NSLOT - 1) if L1 is None else L1
        assert LOOK <= NSLOT - 1 and LK <= LOOK and LV <= LOOK
        sizes = [int(ch) for ch in scheme]
        assert sum(sizes) == CB and all(s % 2 == 0 for s in sizes)
        ends = list(np.cumsum(sizes))
        SRL = sizes[-1] * Sq

        def kernel(x_hbm, k_hbm, v_hbm, wq_hbm, wo_hbm, o_hbm,
                   kb, vb, xb, wb, q_s, o_s, acc_s, ob, s_a, s_b, m_a, m_b,
                   ksem, vsem, wqsem, wosem, xsem, osem, zs):
            def scope(name):
                return jax.named_scope(name) if scopes else contextlib.nullcontext()

            class Tie:
                def __init__(self):
                    self.z = 0
                def off(self, r0):
                    return pl.multiple_of(r0 + self.z, 16)
                def after(self, sems, idx):
                    if tie:
                        self.z = self.z + pl.semaphore_read(sems.at[idx])
                        if CH_S:
                            w = zs[0]
                            for _ in range(CH_S):
                                self.z = (self.z ^ w) + w

            def part(hbm, buf, sem, i, r0, n):
                g = i // B
                b = i % B
                slot = i % NSLOT
                return pltpu.make_async_copy(hbm.at[b, g, pl.ds(r0, n)], buf.at[slot, pl.ds(r0, n)], sem.at[slot])

            def k_all(slot):
                return pltpu.make_async_copy(kb.at[slot], kb.at[slot], ksem.at[slot])

            def v_all(slot):
                return pltpu.make_async_copy(vb.at[slot], vb.at[slot], vsem.at[slot])

            def wq_copy(g):
                return pltpu.make_async_copy(wq_hbm.at[:, pl.ds(pl.multiple_of(g * G, G), G)], wb.at[g], wqsem.at[g])

            def wo_copy(g):
                return pltpu.make_async_copy(wo_hbm.at[pl.ds(pl.multiple_of(g * G, G), G), :], wb.at[Hkv + g % 2], wosem.at[g % 2])

            def out_copy(r0, n, s):
                return pltpu.make_async_copy(ob.at[pl.ds(r0, n), :], o_hbm.at[pl.ds(r0, n), :], osem.at[s])

            cx = pltpu.make_async_copy(x_hbm, xb, xsem.at[0])
            cx.start(priority=1)

            def w_fill(g, _):
                wq_copy(g).start(priority=1)
                zs[g] = 0
                return 0
            jax.lax.fori_loop(0, Hkv if not WQP else 1, w_fill, 0)
            if WQP:
                def z_fill(g, _):
                    zs[g] = 0
                    return 0
                jax.lax.fori_loop(1, Hkv, z_fill, 0)

            def fill(i, _):
                @pl.when(i < LK)
                def _():
                    part(k_hbm, kb, ksem, i, 0, Sk).start(priority=1)
                @pl.when(i >= LK)
                def _():
                    if kbig: part(k_hbm, kb, ksem, i, 0, kbig).start(priority=1)
                @pl.when(i < LV)
                def _():
                    part(v_hbm, vb, vsem, i, 0, Sk).start(priority=1)
                @pl.when(i >= LV)
                def _():
                    if vbig: part(v_hbm, vb, vsem, i, 0, vbig).start(priority=1)
                return 0
            jax.lax.fori_loop(0, wo0_after, fill, 0)
            if not WQP:
                wo_copy(0).start(priority=1)
            jax.lax.fori_loop(wo0_after, LOOK, fill, 0)

            acc_s[...] = jnp.zeros_like(acc_s)
            cx.wait()

            def qproj(g, _):
                pltpu.make_async_copy(wb.at[g], wb.at[g], wqsem.at[g]).wait()
                if not WQP:
                    q = jnp.dot(xb[...], wb[g], preferred_element_type=jnp.float32)
                    q_s[g] = (q * qscale).astype(jnp.bfloat16)
                    return 0
                qn, qm = G // QN, M // QM
                npc = QN * QM * QPP
                wr = D // npc
                for n in range(QN):
                    for mi in range(QM):
                        for t in range(QPP):
                            w0 = ((n * QM + mi) * QPP + t) * wr
                            @pl.when(g + 1 < Hkv)
                            def _(w0=w0):
                                pltpu.make_async_copy(wq_hbm.at[pl.ds(w0, wr), pl.ds(pl.multiple_of((g + 1) * G, G), G)],
                                                      wb.at[g + 1, pl.ds(w0, wr), :], wqsem.at[g + 1]).start(priority=0)
                            @pl.when(g + 1 == Hkv)
                            def _(w0=w0):
                                pltpu.make_async_copy(wo_hbm.at[pl.ds(w0, wr), :],
                                                      wb.at[Hkv, pl.ds(w0, wr), :], wosem.at[0]).start(priority=0)
                        q = jnp.dot(xb[mi * qm:(mi + 1) * qm, :], wb[g, :, n * qn:(n + 1) * qn], preferred_element_type=jnp.float32)
                        q_s[g, mi * qm:(mi + 1) * qm, n * qn:(n + 1) * qn] = (q * qscale).astype(jnp.bfloat16)
                return 0
            jax.lax.fori_loop(0, Hkv, qproj, 0)

            def stage_a_gen(i, s_buf, m_buf, k_piece, big=None):
                g = i // B
                b = i % B
                slot = i % NSLOT
                row0 = pl.multiple_of(b * Sq, Sq)
                qq = jnp.concatenate([q_s[g, pl.ds(row0, Sq), h * Dh:(h + 1) * Dh] for h in range(rep)], axis=0)
                ck = Sk // SCH
                mm = None
                for c in range(SCH):
                    if kpos == 'before':
                        for j in range(c * NPK // SCH, (c + 1) * NPK // SCH):
                            k_piece(j)
                    s = jax.lax.dot_general(qq, kb[slot, c * ck:(c + 1) * ck, :], (((1,), (1,)), ((), ())), preferred_element_type=jnp.float32)
                    s_buf[:, c * ck:(c + 1) * ck] = s
                    for t in range(ck // 128):
                        st = s[:, t * 128:(t + 1) * 128]
                        mm = st if mm is None else jnp.maximum(mm, st)
                    if big is not None and c == min(bigpos, SCH - 1):
                        big()
                    if kpos == 'after':
                        for j in range(c * NPK // SCH, (c + 1) * NPK // SCH):
                            k_piece(j)
                    if c < SCH - 1:
                        yield
                m = jnp.max(mm, axis=1, keepdims=True)
                m_buf[...] = jnp.broadcast_to(m, (R, 128))

            def stage_b_gen(i, s_buf, m_buf, v_piece, big=None):
                b = i % B
                slot = i % NSLOT
                cp = Sk // PCH
                m = m_buf[...]
                o = None
                lacc = None
                for c in range(PCH):
                    ps = []
                    for t in range(cp // 128):
                        c0 = c * cp + t * 128
                        p = jnp.exp2(s_buf[:, c0:c0 + 128] - m)
                        lacc = p if lacc is None else lacc + p
                        ps.append(p.astype(jnp.bfloat16))
                    pc = jnp.concatenate(ps, axis=1) if len(ps) > 1 else ps[0]
                    if vpos == 'before':
                        for j in range(c * NPV // PCH, (c + 1) * NPV // PCH):
                            v_piece(j)
                    oc = jnp.dot(pc, vb[slot, c * cp:(c + 1) * cp, :], preferred_element_type=jnp.float32)
                    o = oc if o is None else o + oc
                    if big is not None and c == min(bigpos, PCH - 1):
                        big()
                    if vpos == 'after':
                        for j in range(c * NPV // PCH, (c + 1) * NPV // PCH):
                            v_piece(j)
                    if c < PCH - 1:
                        yield
                l = jnp.sum(lacc, axis=1, keepdims=True)
                o = o * pl.reciprocal(l, approx=False)
                ob_ = o.astype(jnp.bfloat16)
                orow = pl.multiple_of((b % CB) * Sq, Sq)
                for h in range(rep):
                    o_s[pl.ds(orow, Sq), h * Dh:(h + 1) * Dh] = ob_[h * Sq:(h + 1) * Sq, :]

            def run_all(*gens):
                gens = list(gens)
                while gens:
                    for gq in list(gens):
                        try:
                            next(gq)
                        except StopIteration:
                            gens.remove(gq)

            def step(i, s_cur, m_cur, s_nxt, m_nxt, only_b=False):
                ia = jnp.minimum(i + 1, N - 1)
                NN = N if not nodma else 0

                tz = Tie()

                def k_piece(j):
                    r0 = tz.off(kbig + j * PROW)
                    @pl.when(i + LK < NN)
                    def _():
                        part(k_hbm, kb, ksem, i + LK, r0, PROW).start(priority=0)
                    tz.after(ksem, NSLOT)

                def v_piece(j):
                    r0 = tz.off(vbig + j * PROW)
                    @pl.when(i + LV < NN)
                    def _():
                        part(v_hbm, vb, vsem, i + LV, r0, PROW).start(priority=0)
                    tz.after(vsem, NSLOT)

                if not nodma:
                    with scope("wk"):
                        @pl.when(i + 1 < N)
                        def _():
                            k_all((i + 1) % NSLOT).wait()
                    with scope("wv"):
                        v_all(i % NSLOT).wait()

                def big_k():
                    @pl.when(i + LOOK < NN)
                    def _():
                        if kbig: part(k_hbm, kb, ksem, i + LOOK, 0, kbig).start(priority=1)

                def big_v():
                    @pl.when(i + LOOK < NN)
                    def _():
                        if vbig: part(v_hbm, vb, vsem, i + LOOK, 0, vbig).start(priority=1)

                if bigpos < 0:
                    big_k(); big_v()
                ga = stage_a_gen(ia, s_nxt, m_nxt, k_piece, big_k if bigpos >= 0 else None)
                gb = stage_b_gen(i, s_cur, m_cur, v_piece, big_v if bigpos >= 0 else None)
                if only_b:
                    run_all(stage_b_gen(i, s_cur, m_cur, lambda j: None, None))
                elif order == "AB":
                    run_all(ga); run_all(gb)
                elif order == "BA":
                    run_all(gb); run_all(ga)
                elif order == "IAB":
                    run_all(ga, gb)
                else:
                    run_all(gb, ga)

            k_all(0).wait()
            run_all(stage_a_gen(0, s_a, m_a, lambda j: None))

            def duo(d, _):
                i0 = d * 2
                g = i0 // B
                b1 = i0 % B + 1

                if not WOP:
                    @pl.when((b1 == wo_at + 1) & (g + 1 < Hkv))
                    def _():
                        wo_copy(g + 1).start(priority=1)

                @pl.when(d == N // 2 - 1)
                def _():
                    out_copy(0, M - SRL, 0).start()

                step(i0, s_a, m_a, s_b, m_b)
                if not blast:
                    step(i0 + 1, s_b, m_b, s_a, m_a)
                else:
                    @pl.when(d < N // 2 - 1)
                    def _():
                        step(i0 + 1, s_b, m_b, s_a, m_a)
                    @pl.when(d == N // 2 - 1)
                    def _():
                        step(i0 + 1, s_b, m_b, s_a, m_a, only_b=True)

                @pl.when(b1 == CB - 1)
                def _():
                    pltpu.make_async_copy(wb.at[Hkv + g % 2], wb.at[Hkv + g % 2], wosem.at[g % 2]).wait()

                last_chunk = i0 >= N - CB
                with scope("oproj"):
                    @pl.when((b1 % CB == CB - 1) & jnp.logical_not(last_chunk))
                    def _():
                        c = b1 // CB
                        r0 = pl.multiple_of(c * CR, CR)
                        if not WOP:
                            a = acc_s[pl.ds(r0, CR), :] + jnp.dot(o_s[...], wb[Hkv + g % 2], preferred_element_type=jnp.float32)
                            acc_s[pl.ds(r0, CR), :] = a
                            ob[pl.ds(r0, CR), :] = a.astype(ob.dtype)
                        else:
                            nw = D // ON
                            wr = G // (B // CB) // (ON * OPP)
                            for n in range(ON):
                                for t in range(OPP):
                                    @pl.when(g + 1 < Hkv)
                                    def _(n=n, t=t):
                                        w0 = pl.multiple_of((c * ON * OPP + n * OPP + t) * wr, wr)
                                        pltpu.make_async_copy(wo_hbm.at[pl.ds((g + 1) * G + w0, wr), :],
                                                              wb.at[Hkv + (g + 1) % 2, pl.ds(w0, wr), :],
                                                              wosem.at[(g + 1) % 2]).start(priority=0)
                                a = acc_s[pl.ds(r0, CR), n * nw:(n + 1) * nw] + jnp.dot(
                                    o_s[...], wb[Hkv + g % 2, :, n * nw:(n + 1) * nw], preferred_element_type=jnp.float32)
                                acc_s[pl.ds(r0, CR), n * nw:(n + 1) * nw] = a
                                ob[pl.ds(r0, CR), n * nw:(n + 1) * nw] = a.astype(ob.dtype)

                    for sz in sorted(set(sizes)):
                        cond = None
                        for s_, e_ in zip(sizes, ends):
                            if s_ == sz:
                                c_ = (i0 + 2 == N - CB + int(e_))
                                cond = c_ if cond is None else (cond | c_)

                        def small(sz=sz):
                            nr = sz * Sq
                            r0 = pl.multiple_of((b1 + 1 - sz) * Sq, 2 * Sq)
                            rs = pl.multiple_of(((b1 + 1 - sz) % CB) * Sq, 2 * Sq)
                            a = acc_s[pl.ds(r0, nr), :] + jnp.dot(o_s[pl.ds(rs, nr), :], wb[Hkv + (Hkv - 1) % 2], preferred_element_type=jnp.float32)
                            ob[pl.ds(r0, nr), :] = a.astype(ob.dtype)
                        pl.when(cond)(small)
                return 0

            jax.lax.fori_loop(0, N // 2, duo, 0)
            c2 = out_copy(M - SRL, SRL, 1)
            c2.start()
            out_copy(0, M - SRL, 0).wait()
            c2.wait()

        out = pl.pallas_call(
            kernel,
            in_specs=[pl.BlockSpec(memory_space=pl.ANY)] * 5,
            out_specs=pl.BlockSpec(memory_space=pl.ANY),
            out_shape=jax.ShapeDtypeStruct((M, D), x.dtype),
            scratch_shapes=[
                pltpu.VMEM((NSLOT, Sk, Dh), jnp.bfloat16),
                pltpu.VMEM((NSLOT, Sk, Dh), jnp.bfloat16),
                pltpu.VMEM((M, D), jnp.bfloat16),
                pltpu.VMEM((Hkv + 2, D, G), jnp.bfloat16),
                pltpu.VMEM((Hkv, M, G), jnp.bfloat16),
                pltpu.VMEM((CR, G), jnp.bfloat16),
                pltpu.VMEM((M, D), jnp.float32),
                pltpu.VMEM((M, D), jnp.bfloat16),
                pltpu.VMEM((R, Sk), jnp.float32),
                pltpu.VMEM((R, Sk), jnp.float32),
                pltpu.VMEM((R, 128), jnp.float32),
                pltpu.VMEM((R, 128), jnp.float32),
                pltpu.SemaphoreType.DMA((NSLOT + 1,)),
                pltpu.SemaphoreType.DMA((NSLOT + 1,)),
                pltpu.SemaphoreType.DMA((Hkv,)),
                pltpu.SemaphoreType.DMA((3,)),
                pltpu.SemaphoreType.DMA((1,)),
                pltpu.SemaphoreType.DMA((2,)),
                pltpu.SMEM((Hkv,), jnp.int32),
            ],
            compiler_params=pltpu.CompilerParams(vmem_limit_bytes=110 * 1024 * 1024, disable_bounds_checks=nobc),
        )(x.reshape(M, D), k_cache, v_cache, wq, wo)
        return out.reshape(B, Sq, D)
    return fn

pallas_standalone__gqa_block_cached__sampling_kernel = jax.jit(make(bigpos=3, QM=4, QPP=2))
```

```python
import jax
import jax.numpy as jnp
import jax.experimental.pallas as pl
import jax.experimental.pallas.tpu as pltpu

LOG2E = 1.4426950408889634

NSLOT = 16
NSEM = 16
LOOK = 13
LOOK_K = 3
LOOK_V = 2
PRE = 8
PROW = 128
NPK = 3
NPV = 7
NCHUNK = 8
KSKIP = 5
VSKIP = 1
QN, QM = 8, 4
ON = 8
TAIL = (4, 2, 2)
OUT_CHUNK = 8


def _interleave(*gens):
    gens = list(gens)
    end = object()
    while gens:
        gens = [g for g in gens if next(g, end) is not end]


@jax.jit
def pallas_standalone__gqa_block_cached__sampling_kernel(
    x: jax.Array,
    k_cache: jax.Array,
    v_cache: jax.Array,
    wq: jax.Array,
    wo: jax.Array,
):
    B, Sq, D = x.shape
    _, Hkv, Sk, Dh = k_cache.shape
    Hq = wq.shape[1] // Dh
    rep = Hq // Hkv
    G = rep * Dh
    M = B * Sq
    R = rep * Sq
    N = B * Hkv
    CB = OUT_CHUNK
    CR = CB * Sq
    NCH = B // CB
    CK = Sk // NCHUNK
    kbig = Sk - NPK * PROW
    vbig = Sk - NPV * PROW
    qscale = float(Dh ** -0.5 * LOG2E)
    tail_end = [sum(TAIL[:j + 1]) for j in range(len(TAIL))]
    n_tail = tail_end[-1]
    last_rows = TAIL[-1] * Sq
    WO0 = Hkv

    def kernel(x_hbm, k_hbm, v_hbm, wq_hbm, wo_hbm, o_hbm,
               kb, vb, xb, wb, q_s, o_s, acc_s, ob, s_a, s_b, m_a, m_b, kvsem, wsem):

        def k_sem(i):
            return kvsem.at[(i + NSEM - 1) % NSEM]

        def v_sem(i):
            return kvsem.at[i % NSEM]

        def k_part(i, r0, n):
            return pltpu.make_async_copy(k_hbm.at[i % B, i // B, pl.ds(r0, n)], kb.at[i % NSLOT, pl.ds(r0, n)], k_sem(i))

        def v_part(i, r0, n):
            return pltpu.make_async_copy(v_hbm.at[i % B, i // B, pl.ds(r0, n)], vb.at[i % NSLOT, pl.ds(r0, n)], v_sem(i))

        def k_wait(i):
            pltpu.make_async_copy(kb.at[i % NSLOT], kb.at[i % NSLOT], k_sem(i)).wait()

        def v_wait(i):
            pltpu.make_async_copy(vb.at[i % NSLOT], vb.at[i % NSLOT], v_sem(i)).wait()

        def w_wait(block, sem):
            pltpu.make_async_copy(wb.at[block], wb.at[block], wsem.at[sem]).wait()

        def out_copy(r0, n, sem):
            return pltpu.make_async_copy(ob.at[pl.ds(r0, n), :], o_hbm.at[pl.ds(r0, n), :], wsem.at[sem])

        x_copy = pltpu.make_async_copy(x_hbm, xb, wsem.at[1])

        def first_fetch(t, carry):
            @pl.when(t == 0)
            def _():
                x_copy.start(priority=1)

            @pl.when(t == 1)
            def _():
                pltpu.make_async_copy(wq_hbm.at[:, pl.ds(0, G)], wb.at[0], wsem.at[0]).start(priority=1)
            return carry
        jax.lax.fori_loop(0, 2, first_fetch, 0)

        def ring_fill(i, carry):
            @pl.when(i < PRE)
            def _():
                k_part(i, 0, Sk).start(priority=1)
                v_part(i, 0, Sk).start(priority=1)

            @pl.when(i >= PRE)
            def _():
                k_part(i, 0, kbig).start(priority=1)
                v_part(i, 0, vbig).start(priority=1)
            return carry
        jax.lax.fori_loop(0, LOOK, ring_fill, 0)

        acc_s[...] = jnp.zeros_like(acc_s)
        x_copy.wait()

        def q_proj(g, carry):
            w_wait(g, g % 2)
            qn, qm = G // QN, M // QM
            wr = D // (QN * QM)
            for n in range(QN):
                for mi in range(QM):
                    w0 = (n * QM + mi) * wr

                    @pl.when(g + 1 < Hkv)
                    def _(w0=w0):
                        pltpu.make_async_copy(wq_hbm.at[pl.ds(w0, wr), pl.ds(pl.multiple_of((g + 1) * G, G), G)],
                                              wb.at[g + 1, pl.ds(w0, wr), :], wsem.at[(g + 1) % 2]).start(priority=0)

                    @pl.when(g + 1 == Hkv)
                    def _(w0=w0):
                        pltpu.make_async_copy(wo_hbm.at[pl.ds(w0, wr), :],
                                              wb.at[WO0, pl.ds(w0, wr), :], wsem.at[WO0 % 2]).start(priority=0)

                    q = jnp.dot(xb[mi * qm:(mi + 1) * qm, :], wb[g, :, n * qn:(n + 1) * qn],
                                preferred_element_type=jnp.float32)
                    q_s[g, mi * qm:(mi + 1) * qm, n * qn:(n + 1) * qn] = (q * qscale).astype(jnp.bfloat16)
            return carry
        jax.lax.fori_loop(0, Hkv, q_proj, 0)

        def stage_a(i, s_buf, m_buf, after_chunk):
            g, b, slot = i // B, i % B, i % NSLOT
            row0 = pl.multiple_of(b * Sq, Sq)
            q = jnp.concatenate([q_s[g, pl.ds(row0, Sq), h * Dh:(h + 1) * Dh] for h in range(rep)], axis=0)
            mm = None
            for c in range(NCHUNK):
                s = jax.lax.dot_general(q, kb[slot, c * CK:(c + 1) * CK, :], (((1,), (1,)), ((), ())),
                                        preferred_element_type=jnp.float32)
                s_buf[:, c * CK:(c + 1) * CK] = s
                for t in range(CK // 128):
                    st = s[:, t * 128:(t + 1) * 128]
                    mm = st if mm is None else jnp.maximum(mm, st)
                after_chunk(c)
                if c < NCHUNK - 1:
                    yield
            m_buf[...] = jnp.broadcast_to(jnp.max(mm, axis=1, keepdims=True), (R, 128))

        def stage_b(i, s_buf, m_buf, after_chunk):
            b, slot = i % B, i % NSLOT
            m = m_buf[...]
            o = None
            lsum = None
            for c in range(NCHUNK):
                ps = []
                for t in range(CK // 128):
                    c0 = c * CK + t * 128
                    p = jnp.exp2(s_buf[:, c0:c0 + 128] - m)
                    lsum = p if lsum is None else lsum + p
                    ps.append(p.astype(jnp.bfloat16))
                oc = jnp.dot(jnp.concatenate(ps, axis=1), vb[slot, c * CK:(c + 1) * CK, :],
                             preferred_element_type=jnp.float32)
                o = oc if o is None else o + oc
                after_chunk(c)
                if c < NCHUNK - 1:
                    yield
            l = jnp.sum(lsum, axis=1, keepdims=True)
            o = (o * pl.reciprocal(l, approx=False)).astype(jnp.bfloat16)
            orow = pl.multiple_of((b % CB) * Sq, Sq)
            for h in range(rep):
                o_s[pl.ds(orow, Sq), h * Dh:(h + 1) * Dh] = o[h * Sq:(h + 1) * Sq, :]

        def no_op(c):
            del c

        def step(i, s_cur, m_cur, s_nxt, m_nxt):
            k_wait(i + 1)
            v_wait(i)

            def after_a(c):
                if c == NCHUNK - 1:
                    @pl.when(i + LOOK < N)
                    def _():
                        k_part(i + LOOK, 0, kbig).start(priority=1)
                if c >= KSKIP:
                    n = NCHUNK - KSKIP
                    for j in range((c - KSKIP) * NPK // n, (c - KSKIP + 1) * NPK // n):
                        @pl.when((i + LOOK_K < N) & (i + LOOK_K >= PRE))
                        def _(j=j):
                            k_part(i + LOOK_K, kbig + j * PROW, PROW).start(priority=0)

            def after_b(c):
                if c == NCHUNK - 1:
                    @pl.when(i + LOOK < N)
                    def _():
                        v_part(i + LOOK, 0, vbig).start(priority=1)
                if c >= VSKIP:
                    n = NCHUNK - VSKIP
                    for j in range((c - VSKIP) * NPV // n, (c - VSKIP + 1) * NPV // n):
                        @pl.when((i + LOOK_V < N) & (i + LOOK_V >= PRE))
                        def _(j=j):
                            v_part(i + LOOK_V, vbig + j * PROW, PROW).start(priority=0)

            _interleave(stage_a(i + 1, s_nxt, m_nxt, after_a), stage_b(i, s_cur, m_cur, after_b))

        def out_proj_tail(b_last, nb):
            nr = nb * Sq
            r0 = pl.multiple_of((b_last + 1 - nb) * Sq, 2 * Sq)
            rs = pl.multiple_of(((b_last + 1 - nb) % CB) * Sq, 2 * Sq)
            a = acc_s[pl.ds(r0, nr), :] + jnp.dot(o_s[pl.ds(rs, nr), :], wb[WO0 + (Hkv - 1) % 2],
                                                  preferred_element_type=jnp.float32)
            ob[pl.ds(r0, nr), :] = a.astype(ob.dtype)

        def out_proj(g, c):
            r0 = pl.multiple_of(c * CR, CR)
            nw = D // ON
            wr = G // (NCH * ON)
            for n in range(ON):
                @pl.when(g + 1 < Hkv)
                def _(n=n):
                    w0 = pl.multiple_of((c * ON + n) * wr, wr)
                    pltpu.make_async_copy(wo_hbm.at[pl.ds((g + 1) * G + w0, wr), :],
                                          wb.at[WO0 + (g + 1) % 2, pl.ds(w0, wr), :],
                                          wsem.at[(WO0 + g + 1) % 2]).start(priority=0)

                a = acc_s[pl.ds(r0, CR), n * nw:(n + 1) * nw] + jnp.dot(
                    o_s[...], wb[WO0 + g % 2, :, n * nw:(n + 1) * nw], preferred_element_type=jnp.float32)
                acc_s[pl.ds(r0, CR), n * nw:(n + 1) * nw] = a
                ob[pl.ds(r0, CR), n * nw:(n + 1) * nw] = a.astype(ob.dtype)

        k_wait(0)
        _interleave(stage_a(0, s_a, m_a, no_op))

        def duo(d, carry):
            i0 = d * 2
            g = i0 // B
            b1 = i0 % B + 1
            last = d == N // 2 - 1

            @pl.when(last)
            def _():
                out_copy(0, M - last_rows, 0).start()

            step(i0, s_a, m_a, s_b, m_b)

            @pl.when(jnp.logical_not(last))
            def _():
                step(i0 + 1, s_b, m_b, s_a, m_a)

            @pl.when(last)
            def _():
                v_wait(i0 + 1)
                _interleave(stage_b(i0 + 1, s_b, m_b, no_op))
                out_proj_tail(B - 1, TAIL[-1])

            @pl.when(b1 == CB - 1)
            def _():
                w_wait(WO0 + g % 2, (WO0 + g) % 2)

            @pl.when((b1 % CB == CB - 1) & (i0 < N - n_tail))
            def _():
                out_proj(g, b1 // CB)

            events = list(zip(TAIL, tail_end))[:-1]
            for nb in sorted({e[0] for e in events}):
                cond = None
                for sz, end in events:
                    if sz == nb:
                        hit = i0 + 2 == N - n_tail + end
                        cond = hit if cond is None else cond | hit

                @pl.when(cond)
                def _(nb=nb):
                    out_proj_tail(b1, nb)
            return carry

        jax.lax.fori_loop(0, N // 2, duo, 0)

        tail_copy = out_copy(M - last_rows, last_rows, 1)
        tail_copy.start()
        out_copy(0, M - last_rows, 0).wait()
        tail_copy.wait()

    out = pl.pallas_call(
        kernel,
        in_specs=[pl.BlockSpec(memory_space=pl.ANY)] * 5,
        out_specs=pl.BlockSpec(memory_space=pl.ANY),
        out_shape=jax.ShapeDtypeStruct((M, D), x.dtype),
        scratch_shapes=[
            pltpu.VMEM((NSLOT, Sk, Dh), jnp.bfloat16),
            pltpu.VMEM((NSLOT, Sk, Dh), jnp.bfloat16),
            pltpu.VMEM((M, D), jnp.bfloat16),
            pltpu.VMEM((Hkv + 2, D, G), jnp.bfloat16),
            pltpu.VMEM((Hkv, M, G), jnp.bfloat16),
            pltpu.VMEM((CR, G), jnp.bfloat16),
            pltpu.VMEM((M, D), jnp.float32),
            pltpu.VMEM((M, D), jnp.bfloat16),
            pltpu.VMEM((R, Sk), jnp.float32),
            pltpu.VMEM((R, Sk), jnp.float32),
            pltpu.VMEM((R, 128), jnp.float32),
            pltpu.VMEM((R, 128), jnp.float32),
            pltpu.SemaphoreType.DMA((NSEM,)),
            pltpu.SemaphoreType.DMA((2,)),
        ],
        compiler_params=pltpu.CompilerParams(vmem_limit_bytes=100 * 1024 * 1024),
    )(x.reshape(M, D), k_cache, v_cache, wq, wo)
    return out.reshape(B, Sq, D)
```

```python
import jax
import jax.numpy as jnp
import jax.experimental.pallas as pl
import jax.experimental.pallas.tpu as pltpu

LOG2E = 1.4426950408889634

NSLOT = 16
NSEM = 16
LOOK = 13
LOOK_K = 3
LOOK_V = 2
PRE = 8
PROW = 128
NPK = 3
NPV = 7
NCHUNK = 8
KSKIP = 5
VSKIP = 1
QN, QM = 8, 4
ON = 8
TAIL = (4, 4)
OUT_CHUNK = 8


def _interleave(*gens):
    gens = list(gens)
    end = object()
    while gens:
        gens = [g for g in gens if next(g, end) is not end]


@jax.jit
def pallas_standalone__gqa_block_cached__sampling_kernel(
    x: jax.Array,
    k_cache: jax.Array,
    v_cache: jax.Array,
    wq: jax.Array,
    wo: jax.Array,
):
    B, Sq, D = x.shape
    _, Hkv, Sk, Dh = k_cache.shape
    Hq = wq.shape[1] // Dh
    rep = Hq // Hkv
    G = rep * Dh
    M = B * Sq
    R = rep * Sq
    N = B * Hkv
    CB = OUT_CHUNK
    CR = CB * Sq
    NCH = B // CB
    CK = Sk // NCHUNK
    kbig = Sk - NPK * PROW
    vbig = Sk - NPV * PROW
    qscale = float(Dh ** -0.5 * LOG2E)
    tail_end = [sum(TAIL[:j + 1]) for j in range(len(TAIL))]
    n_tail = tail_end[-1]
    last_rows = TAIL[-1] * Sq
    WO0 = Hkv

    def kernel(x_hbm, k_hbm, v_hbm, wq_hbm, wo_hbm, o_hbm,
               kb, vb, xb, wb, q_s, o_s, acc_s, ob, s_a, s_b, m_a, m_b, kvsem, wsem):

        def k_sem(i):
            return kvsem.at[(i + NSEM - 1) % NSEM]

        def v_sem(i):
            return kvsem.at[i % NSEM]

        def k_part(i, r0, n):
            return pltpu.make_async_copy(k_hbm.at[i % B, i // B, pl.ds(r0, n)], kb.at[i % NSLOT, pl.ds(r0, n)], k_sem(i))

        def v_part(i, r0, n):
            return pltpu.make_async_copy(v_hbm.at[i % B, i // B, pl.ds(r0, n)], vb.at[i % NSLOT, pl.ds(r0, n)], v_sem(i))

        def k_wait(i):
            pltpu.make_async_copy(kb.at[i % NSLOT], kb.at[i % NSLOT], k_sem(i)).wait()

        def v_wait(i):
            pltpu.make_async_copy(vb.at[i % NSLOT], vb.at[i % NSLOT], v_sem(i)).wait()

        def w_wait(block, sem):
            pltpu.make_async_copy(wb.at[block], wb.at[block], wsem.at[sem]).wait()

        def out_copy(r0, n, sem):
            return pltpu.make_async_copy(ob.at[pl.ds(r0, n), :], o_hbm.at[pl.ds(r0, n), :], wsem.at[sem])

        x_copy = pltpu.make_async_copy(x_hbm, xb, wsem.at[1])

        def first_fetch(t, carry):
            @pl.when(t == 0)
            def _():
                x_copy.start(priority=1)

            @pl.when(t == 1)
            def _():
                pltpu.make_async_copy(wq_hbm.at[:, pl.ds(0, G)], wb.at[0], wsem.at[0]).start(priority=1)
            return carry
        jax.lax.fori_loop(0, 2, first_fetch, 0)

        def ring_fill(i, carry):
            @pl.when(i < PRE)
            def _():
                k_part(i, 0, Sk).start(priority=1)
                v_part(i, 0, Sk).start(priority=1)

            @pl.when(i >= PRE)
            def _():
                k_part(i, 0, kbig).start(priority=1)
                v_part(i, 0, vbig).start(priority=1)
            return carry
        jax.lax.fori_loop(0, LOOK, ring_fill, 0)

        acc_s[...] = jnp.zeros_like(acc_s)
        x_copy.wait()

        def q_proj(g, carry):
            w_wait(g, g % 2)
            qn, qm = G // QN, M // QM
            wr = D // (QN * QM)
            for n in range(QN):
                for mi in range(QM):
                    w0 = (n * QM + mi) * wr

                    @pl.when(g + 1 < Hkv)
                    def _(w0=w0):
                        pltpu.make_async_copy(wq_hbm.at[pl.ds(w0, wr), pl.ds(pl.multiple_of((g + 1) * G, G), G)],
                                              wb.at[g + 1, pl.ds(w0, wr), :], wsem.at[(g + 1) % 2]).start(priority=0)

                    @pl.when(g + 1 == Hkv)
                    def _(w0=w0):
                        pltpu.make_async_copy(wo_hbm.at[pl.ds(w0, wr), :],
                                              wb.at[WO0, pl.ds(w0, wr), :], wsem.at[WO0 % 2]).start(priority=0)

                    q = jnp.dot(xb[mi * qm:(mi + 1) * qm, :], wb[g, :, n * qn:(n + 1) * qn],
                                preferred_element_type=jnp.float32)
                    q_s[g, mi * qm:(mi + 1) * qm, n * qn:(n + 1) * qn] = (q * qscale).astype(jnp.bfloat16)
            return carry
        jax.lax.fori_loop(0, Hkv, q_proj, 0)

        def stage_a(i, s_buf, m_buf, after_chunk):
            g, b, slot = i // B, i % B, i % NSLOT
            row0 = pl.multiple_of(b * Sq, Sq)
            q = jnp.concatenate([q_s[g, pl.ds(row0, Sq), h * Dh:(h + 1) * Dh] for h in range(rep)], axis=0)
            mm = None
            for c in range(NCHUNK):
                s = jax.lax.dot_general(q, kb[slot, c * CK:(c + 1) * CK, :], (((1,), (1,)), ((), ())),
                                        preferred_element_type=jnp.float32)
                s_buf[:, c * CK:(c + 1) * CK] = s
                for t in range(CK // 128):
                    st = s[:, t * 128:(t + 1) * 128]
                    mm = st if mm is None else jnp.maximum(mm, st)
                after_chunk(c)
                if c < NCHUNK - 1:
                    yield
            m_buf[...] = jnp.broadcast_to(jnp.max(mm, axis=1, keepdims=True), (R, 128))

        def stage_b(i, s_buf, m_buf, after_chunk):
            b, slot = i % B, i % NSLOT
            m = m_buf[...]
            o = None
            lsum = None
            for c in range(NCHUNK):
                ps = []
                for t in range(CK // 128):
                    c0 = c * CK + t * 128
                    p = jnp.exp2(s_buf[:, c0:c0 + 128] - m)
                    lsum = p if lsum is None else lsum + p
                    ps.append(p.astype(jnp.bfloat16))
                oc = jnp.dot(jnp.concatenate(ps, axis=1), vb[slot, c * CK:(c + 1) * CK, :],
                             preferred_element_type=jnp.float32)
                o = oc if o is None else o + oc
                after_chunk(c)
                if c < NCHUNK - 1:
                    yield
            l = jnp.sum(lsum, axis=1, keepdims=True)
            o = (o * pl.reciprocal(l, approx=False)).astype(jnp.bfloat16)
            orow = pl.multiple_of((b % CB) * Sq, Sq)
            for h in range(rep):
                o_s[pl.ds(orow, Sq), h * Dh:(h + 1) * Dh] = o[h * Sq:(h + 1) * Sq, :]

        def no_op(c):
            del c

        def step(i, s_cur, m_cur, s_nxt, m_nxt, after_wait=None):
            k_wait(i + 1)
            v_wait(i)
            if after_wait is not None:
                after_wait()

            def after_a(c):
                if c == NCHUNK - 1:
                    @pl.when(i + LOOK < N)
                    def _():
                        k_part(i + LOOK, 0, kbig).start(priority=1)
                if c >= KSKIP:
                    n = NCHUNK - KSKIP
                    for j in range((c - KSKIP) * NPK // n, (c - KSKIP + 1) * NPK // n):
                        @pl.when((i + LOOK_K < N) & (i + LOOK_K >= PRE))
                        def _(j=j):
                            k_part(i + LOOK_K, kbig + j * PROW, PROW).start(priority=0)

            def after_b(c):
                if c == NCHUNK - 1:
                    @pl.when(i + LOOK < N)
                    def _():
                        v_part(i + LOOK, 0, vbig).start(priority=1)
                if c >= VSKIP:
                    n = NCHUNK - VSKIP
                    for j in range((c - VSKIP) * NPV // n, (c - VSKIP + 1) * NPV // n):
                        @pl.when((i + LOOK_V < N) & (i + LOOK_V >= PRE))
                        def _(j=j):
                            v_part(i + LOOK_V, vbig + j * PROW, PROW).start(priority=0)

            _interleave(stage_a(i + 1, s_nxt, m_nxt, after_a), stage_b(i, s_cur, m_cur, after_b))

        def out_proj_tail(b_last, nb):
            nr = nb * Sq
            r0 = pl.multiple_of((b_last + 1 - nb) * Sq, 2 * Sq)
            rs = pl.multiple_of(((b_last + 1 - nb) % CB) * Sq, 2 * Sq)
            a = acc_s[pl.ds(r0, nr), :] + jnp.dot(o_s[pl.ds(rs, nr), :], wb[WO0 + (Hkv - 1) % 2],
                                                  preferred_element_type=jnp.float32)
            ob[pl.ds(r0, nr), :] = a.astype(ob.dtype)

        def out_proj(g, c):
            r0 = pl.multiple_of(c * CR, CR)
            nw = D // ON
            wr = G // (NCH * ON)
            for n in range(ON):
                @pl.when(g + 1 < Hkv)
                def _(n=n):
                    w0 = pl.multiple_of((c * ON + n) * wr, wr)
                    pltpu.make_async_copy(wo_hbm.at[pl.ds((g + 1) * G + w0, wr), :],
                                          wb.at[WO0 + (g + 1) % 2, pl.ds(w0, wr), :],
                                          wsem.at[(WO0 + g + 1) % 2]).start(priority=0)

                a = acc_s[pl.ds(r0, CR), n * nw:(n + 1) * nw] + jnp.dot(
                    o_s[...], wb[WO0 + g % 2, :, n * nw:(n + 1) * nw], preferred_element_type=jnp.float32)
                acc_s[pl.ds(r0, CR), n * nw:(n + 1) * nw] = a
                ob[pl.ds(r0, CR), n * nw:(n + 1) * nw] = a.astype(ob.dtype)

        k_wait(0)
        _interleave(stage_a(0, s_a, m_a, no_op))

        def duo(d, carry):
            i0 = d * 2
            g = i0 // B
            b1 = i0 % B + 1
            last = d == N // 2 - 1

            def flush_output():
                @pl.when(last)
                def _():
                    out_copy(0, M - last_rows, 0).start(priority=1)

            step(i0, s_a, m_a, s_b, m_b, flush_output)

            @pl.when(jnp.logical_not(last))
            def _():
                step(i0 + 1, s_b, m_b, s_a, m_a)

            @pl.when(last)
            def _():
                v_wait(i0 + 1)
                _interleave(stage_b(i0 + 1, s_b, m_b, no_op))
                out_proj_tail(B - 1, TAIL[-1])

            @pl.when(b1 == CB - 1)
            def _():
                w_wait(WO0 + g % 2, (WO0 + g) % 2)

            @pl.when((b1 % CB == CB - 1) & (i0 < N - n_tail))
            def _():
                out_proj(g, b1 // CB)

            events = list(zip(TAIL, tail_end))[:-1]
            for nb in sorted({e[0] for e in events}):
                cond = None
                for sz, end in events:
                    if sz == nb:
                        hit = i0 + 2 == N - n_tail + end
                        cond = hit if cond is None else cond | hit

                @pl.when(cond)
                def _(nb=nb):
                    out_proj_tail(b1, nb)
            return carry

        jax.lax.fori_loop(0, N // 2, duo, 0)

        tail_copy = out_copy(M - last_rows, last_rows, 1)
        tail_copy.start()
        out_copy(0, M - last_rows, 0).wait()
        tail_copy.wait()

    out = pl.pallas_call(
        kernel,
        in_specs=[pl.BlockSpec(memory_space=pl.ANY)] * 5,
        out_specs=pl.BlockSpec(memory_space=pl.ANY),
        out_shape=jax.ShapeDtypeStruct((M, D), x.dtype),
        scratch_shapes=[
            pltpu.VMEM((NSLOT, Sk, Dh), jnp.bfloat16),
            pltpu.VMEM((NSLOT, Sk, Dh), jnp.bfloat16),
            pltpu.VMEM((M, D), jnp.bfloat16),
            pltpu.VMEM((Hkv + 2, D, G), jnp.bfloat16),
            pltpu.VMEM((Hkv, M, G), jnp.bfloat16),
            pltpu.VMEM((CR, G), jnp.bfloat16),
            pltpu.VMEM((M, D), jnp.float32),
            pltpu.VMEM((M, D), jnp.bfloat16),
            pltpu.VMEM((R, Sk), jnp.float32),
            pltpu.VMEM((R, Sk), jnp.float32),
            pltpu.VMEM((R, 128), jnp.float32),
            pltpu.VMEM((R, 128), jnp.float32),
            pltpu.SemaphoreType.DMA((NSEM,)),
            pltpu.SemaphoreType.DMA((2,)),
        ],
        compiler_params=pltpu.CompilerParams(vmem_limit_bytes=100 * 1024 * 1024),
    )(x.reshape(M, D), k_cache, v_cache, wq, wo)
    return out.reshape(B, Sq, D)
```
